```python
import jax
import jax.numpy as jnp

def _softmax(x, axis=-1):
    return jax.nn.softmax(x, axis=axis)
def _gelu(x):
    return jax.nn.gelu(x, approximate=True)
def _silu(x):
    return jax.nn.silu(x)
def _sigmoid(x):
    return jax.nn.sigmoid(x)
def _layernorm(x, axis=-1, eps=1e-5):
    m = jnp.mean(x, axis=axis, keepdims=True)
    v = jnp.var(x, axis=axis, keepdims=True)
    return (x - m) / jnp.sqrt(v + eps)
def _scatter_add(tgt, idx, src, axis=0):
    return tgt.at[idx].add(src)
def _segment_sum(src, seg, n):
    return jax.ops.segment_sum(src, seg, n)
class _Rng:
    def __init__(self, key):
        self._k = key
    def _next(self):
        self._k, sub = jax.random.split(self._k)
        return sub
    def normal(self, shape):
        return jax.random.normal(self._next(), shape, dtype=jnp.bfloat16)
    def randint(self, lo, hi, shape):
        return jax.random.randint(self._next(), shape, lo, hi, dtype=jnp.int32)
    def uniform(self, shape, lo=0.0, hi=1.0):
        return jax.random.uniform(self._next(), shape, jnp.bfloat16, lo, hi)
    def permutation(self, n):
        return jax.random.permutation(self._next(), n)


kernel_name = 'interleave_layers__grouped_kv_mqa__sliding_local_dilated__prompt'

def setup_inputs():
    _rng = _Rng(jax.random.key(int.from_bytes(__import__("os").urandom(4), "little")))
    _w = (lambda a: (lambda t: t.astype(jnp.bfloat16) if jnp.issubdtype(t.dtype, jnp.floating) else t)(jnp.asarray(a)))
    def _A_setup():
        B, S, D, H = 1, 2048, 1024, 32
        Dh = D // H
        return {
            "x": _w((lambda *s: _rng.normal(s) * 0.05)(B, S, D)),
            "wq": _w((lambda *s: _rng.normal(s) * 0.05)(D, H * Dh)),
            "wk": _w((lambda *s: _rng.normal(s) * 0.05)(D, Dh)),
            "wv": _w((lambda *s: _rng.normal(s) * 0.05)(D, Dh)),
            "wo": _w((lambda *s: _rng.normal(s) * 0.05)(H * Dh, D)),
        }
    _A_in = _A_setup()

    def _B_setup():
        B, S, D = 1, 2048, 1024
        return {
            "x": _w((lambda *s: _rng.normal(s) * 0.05)(B, S, D)),
            "wqkv": _w((lambda *s: _rng.normal(s) * 0.05)(D, 3 * D)),
            "wo": _w((lambda *s: _rng.normal(s) * 0.05)(D, D)),
        }
    _B_in = _B_setup()

    return {
        "A_x": _A_in["x"],
        "A_wq": _A_in["wq"],
        "A_wk": _A_in["wk"],
        "A_wv": _A_in["wv"],
        "A_wo": _A_in["wo"],
        "B_x": _B_in["x"],
        "B_wqkv": _B_in["wqkv"],
        "B_wo": _B_in["wo"],
    }

def reference(A_x, A_wq, A_wk, A_wv, A_wo, B_x, B_wqkv, B_wo):
    def _A_ref(x, wq, wk, wv, wo):
        B, S, D = x.shape
        H = 32
        Dh = D // H
        q = (lambda x, *d: x.transpose(*d))((x @ wq).reshape(B, S, H, Dh), 0, 2, 1, 3)
        k = x @ wk
        v = x @ wv
        scores = jnp.einsum("bhqd,bkd->bhqk", q, k) * (Dh ** -0.5)
        p = _softmax(scores, axis=-1)
        o = jnp.einsum("bhqk,bkd->bhqd", p, v)
        return (lambda x, *d: x.transpose(*d))(o, 0, 2, 1, 3).reshape(B, S, H * Dh) @ wo

    def _B_ref(x, wqkv, wo):
        B, S, D = x.shape
        H = 32; Dh = D // H
        W, dil = 8, 2
        qkv = (lambda x, *d: x.transpose(*d))((x @ wqkv).reshape(B, S, 3, H, Dh), 2, 0, 3, 1, 4)
        q, k, v = qkv[0], qkv[1], qkv[2]
        scale = Dh ** -0.5
        pos = jnp.arange(S)
        off = jnp.arange(W) * dil
        idx = pos[:, None] - off[None, :]
        mask = idx >= 0
        idx_c = jnp.where(mask, idx, 0).reshape(-1)
        kg = k[:, :, idx_c, :].reshape(B, H, S, W, Dh)
        vg = v[:, :, idx_c, :].reshape(B, H, S, W, Dh)
        logits = jnp.einsum("bhsd,bhswd->bhsw", q, kg) * scale
        logits = jnp.where(mask[None, None, :, :], logits, -1e9)
        attn = _softmax(logits, axis=-1)
        o = jnp.einsum("bhsw,bhswd->bhsd", attn, vg)
        return (lambda x, *d: x.transpose(*d))(o, 0, 2, 1, 3).reshape(B, S, D) @ wo

    x = A_x
    x = x + _A_ref(_layernorm(x, axis=-1), A_wq, A_wk, A_wv, A_wo)
    x = x + _B_ref(_layernorm(x, axis=-1), B_wqkv, B_wo)
    x = x + _A_ref(_layernorm(x, axis=-1), A_wq, A_wk, A_wv, A_wo)
    x = x + _B_ref(_layernorm(x, axis=-1), B_wqkv, B_wo)
    return x
```

```python
import jax
import jax.numpy as jnp
from jax import lax
import jax.experimental.pallas as pl
import jax.experimental.pallas.tpu as pltpu

S = 2048
D = 1024
H = 32
DH = D // H
WIN = 8
DIL = 2
EPS = 1e-5
LOG2E = 1.4426950408889634
QSCALE = DH ** -0.5 * LOG2E
MASKED = -1e9 * LOG2E

NQ = 512
NU = S // NQ
KC = 128
NC = S // KC
TB = 128
TS = 64
NB = S // TB
HALO = 16
NT = D // 128

F32 = jnp.float32
BF16 = jnp.bfloat16
U32 = jnp.uint32


def _dot(a, b):
    return jnp.dot(a, b, preferred_element_type=F32)


def _dot_nt(a, b):
    return lax.dot_general(a, b, (((1,), (1,)), ((), ())), preferred_element_type=F32)


def _layernorm(x):
    m = jnp.mean(x, axis=-1, keepdims=True)
    c = x - m
    v = jnp.mean(c * c, axis=-1, keepdims=True)
    return (c * lax.rsqrt(v + EPS)).astype(BF16)


def _kernel(x_hbm, awq_hbm, awkt_hbm, awvt_hbm, awo_hbm, bwqkv_hbm, bwo_hbm, out_hbm,
            xin, xres, awq, awkvt, awo, bwqkv_raw, bwqkv, bwo_raw, bwo,
            q_s, k4_s, vt_s, s_s, m_s, ot_s, o_s, kh_s, vh_s, out_s, tr_s,
            sem_in, sem_out):
    half = S // 2

    def x_copy(i):
        rows = pl.ds(i * half, half)
        return pltpu.make_async_copy(x_hbm.at[rows], xin.at[rows], sem_in.at[i])

    akt_cp = pltpu.make_async_copy(awkt_hbm, awkvt.at[pl.ds(0, DH)], sem_in.at[2])
    avt_cp = pltpu.make_async_copy(awvt_hbm, awkvt.at[pl.ds(DH, DH)], sem_in.at[3])
    awq_cp = pltpu.make_async_copy(awq_hbm, awq, sem_in.at[4])
    awo_cp = pltpu.make_async_copy(awo_hbm, awo, sem_in.at[5])
    bwqkv_cps = [
        pltpu.make_async_copy(bwqkv_hbm.at[:, pl.ds(t * 128, 128)], bwqkv_raw.at[t], sem_in.at[6])
        for t in range(3 * NT)]
    bwo_cps = [
        pltpu.make_async_copy(bwo_hbm.at[:, pl.ds(t * 128, 128)], bwo_raw.at[t], sem_in.at[7])
        for t in range(NT)]

    def out_copy(i, slot):
        return pltpu.make_async_copy(
            out_s.at[slot], out_hbm.at[pl.ds(pl.multiple_of(i * TB, TB), TB)], sem_out.at[slot])

    akt_cp.start()
    avt_cp.start()
    x_copy(0).start()
    awq_cp.start()
    x_copy(1).start()
    awo_cp.start()
    for cp in bwqkv_cps:
        cp.start()
    for cp in bwo_cps:
        cp.start()

    lane = lax.broadcasted_iota(jnp.int32, (TB, 128), 1)

    def project_a(xn, rows):
        kvt = _dot_nt(awkvt[...], xn)
        vt_s[:, rows] = kvt[DH:].astype(BF16)
        krep = jnp.concatenate([kvt[:DH]] * 4, axis=0).T
        for j in range(4):
            k4_s[j, rows, :] = jnp.where(lane // DH == j, krep, 0.0).astype(BF16)
        q_s[rows, :] = (_dot(xn, awq[...]) * QSCALE).astype(BF16)

    akt_cp.wait()
    avt_cp.wait()
    x_copy(0).wait()
    awq_cp.wait()

    def first(i, carry):
        @pl.when(i == NB // 2)
        def _():
            x_copy(1).wait()

        rows = pl.ds(pl.multiple_of(i * TB, TB), TB)
        x = xin[rows, :].astype(F32)
        xres[rows, :] = x
        project_a(_layernorm(x), rows)
        return carry

    lax.fori_loop(0, NB, first, 0)

    awo_cp.wait()
    for cp in bwqkv_cps:
        cp.wait()
    for cp in bwo_cps:
        cp.wait()

    raw32 = bwqkv_raw.bitcast(U32)
    new32 = bwqkv.bitcast(U32)

    def permute_qkv(n, carry):
        sec = n // 4
        r = pl.ds(pl.multiple_of((n % 4) * 128, 128), 128)
        for t in range(NT):
            tr_s[pl.ds(t * 128, 128), :] = raw32[sec * NT + t, r, :].T
        for t in range(NT):
            blk = jnp.concatenate(
                [tr_s[pl.ds(4 * t + e, H, stride=DH), :] for e in range(4)], axis=0)
            new32[r, pl.ds(pl.multiple_of(sec * D + t * 128, 128), 128)] = blk.T
        return carry

    lax.fori_loop(0, 12, permute_qkv, 0)

    wo32 = bwo_raw.bitcast(U32)
    newo32 = bwo.bitcast(U32)
    for t in range(NT):
        cols = pl.ds(t * 128, 128)
        for dp in range(DH // 2):
            ev = wo32[t, pl.ds(dp, H // 2, stride=DH), :]
            od = wo32[t, pl.ds(DH // 2 + dp, H // 2, stride=DH), :]
            newo32[pl.ds(dp * H, H // 2), cols] = (ev & 0xFFFF) | (od << 16)
            newo32[pl.ds(dp * H + H // 2, H // 2), cols] = (ev >> 16) | (od & U32(0xFFFF0000))

    def attention(h_qk, h_pv):
        st = {}

        def scores(t):
            u, c = divmod(t, NC)
            keys = pl.ds(c * KC, KC)
            cols = pl.ds(u * NQ, NQ)
            qcols = pl.ds(pl.multiple_of((h_qk // 4) * 128, 128), 128)
            s = _dot_nt(k4_s[h_qk % 4, keys, :], q_s[cols, qcols])
            s_s[keys, cols] = s
            m = jnp.max(s.reshape(KC // 8, 8, NQ), axis=0)
            st["m"] = m if c == 0 else jnp.maximum(st["m"], m)
            if c == NC - 1:
                m_s[:, cols] = jnp.broadcast_to(
                    jnp.max(st["m"], axis=0, keepdims=True), (8, NQ))

        def values(t):
            u, c = divmod(t, NC)
            keys = pl.ds(c * KC, KC)
            cols = pl.ds(u * NQ, NQ)
            if c == 0:
                st["mp"] = m_s[:, cols]
            p = jnp.exp2(s_s[keys, cols].reshape(KC // 8, 8, NQ) - st["mp"][None])
            l = jnp.sum(p, axis=0)
            o = _dot(vt_s[:, keys], p.reshape(KC, NQ).astype(BF16))
            st["l"] = l if c == 0 else st["l"] + l
            st["o"] = o if c == 0 else st["o"] + o
            if c == NC - 1:
                inv = 1.0 / jnp.sum(st["l"], axis=0, keepdims=True)
                ot_s[pl.ds(pl.multiple_of(h_pv * DH, DH), DH), cols] = (
                    st["o"] * inv).astype(BF16)

        for t in range(NU * NC):
            if h_pv is not None:
                values(t)
            if h_qk is not None:
                scores(t)

    def transpose_o(i):
        rows = pl.ds(pl.multiple_of(i * TB, TB), TB)
        o_s[rows, :] = ot_s[:, rows].T

    def local_attention(q, off, pos0):
        logits = []
        for w in range(WIN):
            src = pl.ds(HALO + off - w * DIL, TS)
            acc = q[0] * kh_s[0, src, :]
            for t in range(1, NT):
                acc = acc + q[t] * kh_s[t, src, :]
            acc = acc + pltpu.roll(acc, 64, 1)
            acc = acc + pltpu.roll(acc, 32, 1)
            if off < w * DIL:
                pos = pos0 + lax.broadcasted_iota(jnp.int32, (HALO, 128), 0)
                head = jnp.where(pos >= w * DIL, acc[:HALO], MASKED)
                acc = jnp.concatenate([head, acc[HALO:]], axis=0)
            logits.append(acc)
        m = logits[0]
        for w in range(1, WIN):
            m = jnp.maximum(m, logits[w])
        p = [jnp.exp2(lg - m) for lg in logits]
        l = p[0]
        for w in range(1, WIN):
            l = l + p[w]
        inv = 1.0 / l
        p = [pw * inv for pw in p]
        out = []
        for t in range(NT):
            acc = p[0] * vh_s[t, pl.ds(HALO + off, TS), :]
            for w in range(1, WIN):
                acc = acc + p[w] * vh_s[t, pl.ds(HALO + off - w * DIL, TS), :]
            out.append(acc.astype(BF16))
        return jnp.concatenate(out, axis=1)

    def layer(li, carry):
        attention(0, None)

        def head(h, c):
            attention(h, h - 1)
            return c

        lax.fori_loop(1, H, head, 0)
        attention(None, H - 1)

        transpose_o(0)

        def block(i, c):
            base = pl.multiple_of(i * TB, TB)
            subs = range(TB // TS)
            rows = [pl.ds(pl.multiple_of(base + a * TS, TS), TS) for a in subs]

            x1 = [xres[rows[a], :] + _dot(o_s[rows[a], :], awo[...]) for a in subs]
            transpose_o(jnp.minimum(i + 1, NB - 1))

            @pl.when(i > 0)
            def _():
                kh_s[:, pl.ds(0, HALO), :] = kh_s[:, pl.ds(TB, HALO), :]
                vh_s[:, pl.ds(0, HALO), :] = vh_s[:, pl.ds(TB, HALO), :]

            qs = []
            for a in subs:
                qkv = _dot(_layernorm(x1[a]), bwqkv[...])
                dst = pl.ds(HALO + a * TS, TS)
                qs.append([qkv[:, t * 128:(t + 1) * 128] * QSCALE for t in range(NT)])
                for t in range(NT):
                    kh_s[t, dst, :] = qkv[:, (NT + t) * 128:(NT + t + 1) * 128]
                    vh_s[t, dst, :] = qkv[:, (2 * NT + t) * 128:(2 * NT + t + 1) * 128]
                if a == 0:
                    @pl.when(i == 0)
                    def _():
                        for t in range(NT):
                            kh_s[t, pl.ds(0, HALO), :] = jnp.zeros((HALO, 128), F32)
                            vh_s[t, pl.ds(0, HALO), :] = jnp.broadcast_to(
                                vh_s[t, pl.ds(HALO, 1), :], (HALO, 128))

            x2 = []
            for a in subs:
                o = local_attention(qs[a], a * TS, base)
                x2.append(x1[a] + _dot(o, bwo[...]))
                xres[rows[a], :] = x2[a]

            @pl.when(li == 0)
            def _():
                xn = jnp.concatenate([_layernorm(v) for v in x2], axis=0)
                project_a(xn, pl.ds(base, TB))

            @pl.when(li == 1)
            def _():
                slot = i % 2

                @pl.when(i >= 2)
                def _():
                    out_copy(i - 2, slot).wait()

                out_s[slot] = xres[pl.ds(base, TB), :].astype(BF16)
                out_copy(i, slot).start()

            return c

        lax.fori_loop(0, NB, block, 0)
        return carry

    lax.fori_loop(0, 2, layer, 0)
    out_copy(NB - 2, 0).wait()
    out_copy(NB - 1, 1).wait()


@jax.jit
def pallas_interleave_layers__grouped_kv_mqa__sliding_local_dilated__prompt_kernel(
    A_x: jax.Array,
    A_wq: jax.Array,
    A_wk: jax.Array,
    A_wv: jax.Array,
    A_wo: jax.Array,
    B_x: jax.Array,
    B_wqkv: jax.Array,
    B_wo: jax.Array,
):
    del B_x
    any_spec = pl.BlockSpec(memory_space=pl.ANY)
    out = pl.pallas_call(
        _kernel,
        in_specs=[any_spec] * 7,
        out_specs=any_spec,
        out_shape=jax.ShapeDtypeStruct((S, D), BF16),
        scratch_shapes=[
            pltpu.VMEM((S, D), BF16),
            pltpu.VMEM((S, D), F32),
            pltpu.VMEM((D, D), BF16),
            pltpu.VMEM((2 * DH, D), BF16),
            pltpu.VMEM((D, D), BF16),
            pltpu.VMEM((3 * NT, D, 128), BF16),
            pltpu.VMEM((D, 3 * D), BF16),
            pltpu.VMEM((NT, D, 128), BF16),
            pltpu.VMEM((D, D), BF16),
            pltpu.VMEM((S, D), BF16),
            pltpu.VMEM((4, S, 128), BF16),
            pltpu.VMEM((DH, S), BF16),
            pltpu.VMEM((S, S), F32),
            pltpu.VMEM((8, S), F32),
            pltpu.VMEM((D, S), BF16),
            pltpu.VMEM((S, D), BF16),
            pltpu.VMEM((NT, HALO + TB, 128), F32),
            pltpu.VMEM((NT, HALO + TB, 128), F32),
            pltpu.VMEM((2, TB, D), BF16),
            pltpu.VMEM((D, 128), U32),
            pltpu.SemaphoreType.DMA((8,)),
            pltpu.SemaphoreType.DMA((2,)),
        ],
        compiler_params=pltpu.CompilerParams(vmem_limit_bytes=120 * 1024 * 1024),
    )(A_x.reshape(S, D), A_wq, A_wk.T, A_wv.T, A_wo, B_wqkv, B_wo)
    return out.reshape(A_x.shape)
```

```python
import jax
import jax.numpy as jnp
from jax import lax
import jax.experimental.pallas as pl
import jax.experimental.pallas.tpu as pltpu

S = 2048
D = 1024
H = 32
DH = D // H
WIN = 8
DIL = 2
EPS = 1e-5
LOG2E = 1.4426950408889634
QSCALE = DH ** -0.5 * LOG2E
MASKED = -1e9 * LOG2E

NQ = 512
NU = S // NQ
KC = 128
NC = S // KC
TF = 128
TB = 256
TS = 64
RT = 16
NB = S // TB
XC = 8
NP = 6
HALO = 16
NT = D // 128
SH = 8 // DIL

F32 = jnp.float32
BF16 = jnp.bfloat16
U32 = jnp.uint32


def _dot(a, b):
    return jnp.dot(a, b, preferred_element_type=F32)


def _dot_nt(a, b):
    return lax.dot_general(a, b, (((1,), (1,)), ((), ())), preferred_element_type=F32)


def _pack(x):
    return pltpu.bitcast(x.astype(BF16), U32)


def _unpack(x):
    return pltpu.bitcast(x, BF16)


def _weights(ref):
    return _unpack(jnp.concatenate([ref[t] for t in range(ref.shape[0])], axis=1))


def _layernorm(x):
    m = jnp.mean(x, axis=-1, keepdims=True)
    c = x - m
    v = jnp.mean(c * c, axis=-1, keepdims=True)
    return (c * lax.rsqrt(v + EPS)).astype(BF16)


def _half(start, size):
    if isinstance(start, int):
        return pl.ds(start // 2, size // 2)
    return pl.ds(pl.multiple_of(start // 2, size // 2), size // 2)


def _kernel(x_hbm, awq_hbm, awkt_hbm, awvt_hbm, awo_hbm, bwqkv_hbm, bwo_hbm, out_hbm,
            xin, xres, xn_s, awq, awkvt, awo, bwqkv_raw, bwqkv, bwo_raw, bwo, tr_s,
            q_s, k4_s, vt_s, s_s, m_s, ot_s, o_s, kh_s, vh_s, out_s,
            sem_in, sem_x, sem_out):
    xc = S // XC

    def x_copy(i):
        rows = pl.ds(i * xc, xc)
        return pltpu.make_async_copy(x_hbm.at[rows], xin.bitcast(BF16).at[rows], sem_x.at[i])

    def tile_copies(src, dst, sem):
        return [pltpu.make_async_copy(src.at[:, pl.ds(t * 128, 128)], dst.bitcast(BF16).at[t], sem)
                for t in range(dst.shape[0])]

    def out_copy(i, slot):
        rows = pl.ds(pl.multiple_of(i * TB, TB), TB)
        return pltpu.make_async_copy(out_s.at[slot], out_hbm.at[rows], sem_out.at[slot])

    akv_cps = [
        pltpu.make_async_copy(src, awkvt.bitcast(BF16).at[pl.ds(e * DH, DH)], sem_in.at[0])
        for e, src in enumerate((awkt_hbm, awvt_hbm))]
    awq_cps = tile_copies(awq_hbm, awq, sem_in.at[1])
    awo_cps = tile_copies(awo_hbm, awo, sem_in.at[2])
    bwqkv_cps = tile_copies(bwqkv_hbm, bwqkv_raw, sem_in.at[3])
    bwo_cps = tile_copies(bwo_hbm, bwo_raw, sem_in.at[4])

    x_copy(0).start()
    for cp in akv_cps + awq_cps:
        cp.start()

    def project_q(xn, base, n):
        q = _pack(_dot(xn, _weights(awq)) * QSCALE)
        for t in range(NT):
            q_s[t, _half(base, n), :] = q[:, t * 128:(t + 1) * 128]

    def project_kv(xn, base, n):
        kvt = _dot_nt(_unpack(awkvt[...]), xn)
        vt_s[:, pl.ds(base, n)] = _pack(kvt[DH:])
        krep = jnp.concatenate([kvt[:DH]] * 4, axis=0).T
        lane = lax.broadcasted_iota(jnp.int32, (n, 128), 1)
        for j in range(4):
            k4_s[j, _half(base, n), :] = _pack(jnp.where(lane // DH == j, krep, 0.0))

    def permute_qkv(n):
        sec = n // 4
        r = pl.ds(pl.multiple_of((n % 4) * 128, 128), 128)
        for t in range(NT):
            tr_s[pl.ds(t * 128, 128), :] = bwqkv_raw[sec * NT + t, r, :].T
        for t in range(NT):
            blk = jnp.concatenate(
                [tr_s[pl.ds(4 * t + e, H, stride=DH), :] for e in range(4)], axis=0)
            bwqkv[sec * NT + t, r, :] = blk.T

    def permute_wo(t, carry):
        for dp in range(DH // 2):
            ev = bwo_raw[t, pl.ds(dp, H // 2, stride=DH), :]
            od = bwo_raw[t, pl.ds(DH // 2 + dp, H // 2, stride=DH), :]
            bwo[t, pl.ds(dp * H, H // 2), :] = (ev & 0xFFFF) | (od << 16)
            bwo[t, pl.ds(dp * H + H // 2, H // 2), :] = (ev >> 16) | (od & U32(0xFFFF0000))
        return carry

    nf = S // TF

    def first_norm(i):
        base = pl.multiple_of(i * TF, TF)
        x = _unpack(xin[_half(base, TF), :]).astype(F32)
        xres[pl.ds(base, TF), :] = x
        xn_s[...] = pltpu.bitcast(_layernorm(x), U32)

    def first(permute, i, carry):
        if not permute:
            for c in range(1, XC):
                @pl.when(i == c * (xc // TF) - 1)
                def _():
                    x_copy(c).wait()

            @pl.when(i == 1)
            def _():
                for cp in bwqkv_cps + bwo_cps + awo_cps:
                    cp.start()

        base = pl.multiple_of(i * TF, TF)
        xn = _unpack(xn_s[...])
        if permute:
            for e in range(12 // NP):
                permute_qkv((i - (nf - NP)) * (12 // NP) + e)
        project_kv(xn, base, TF)
        project_q(xn, base, TF)
        first_norm(jnp.minimum(i + 1, nf - 1))
        return carry

    x_copy(0).wait()
    first_norm(0)
    for cp in akv_cps + awq_cps:
        cp.wait()
    for i in range(1, XC):
        x_copy(i).start()
    lax.fori_loop(0, nf - NP, lambda i, c: first(False, i, c), 0)
    for c in range(1, XC):
        if c * (xc // TF) - 1 >= nf - NP:
            x_copy(c).wait()
    for cp in bwqkv_cps:
        cp.wait()
    lax.fori_loop(nf - NP, nf, lambda i, c: first(True, i, c), 0)
    for cp in bwo_cps + awo_cps:
        cp.wait()
    lax.fori_loop(0, NT, permute_wo, 0)

    def attention(h_qk, h_pv, col0, nu):
        st = {}

        def scores(t):
            u, c = divmod(t, NC)
            q0 = col0 + u * NQ
            s = _dot_nt(_unpack(k4_s[h_qk % 4, _half(c * KC, KC), :]),
                        _unpack(q_s[h_qk // 4, _half(q0, NQ), :]))
            s_s[pl.ds(c * KC, KC), pl.ds(q0, NQ)] = s
            m = jnp.max(s.reshape(KC // 8, 8, NQ), axis=0)
            st["m"] = m if c == 0 else jnp.maximum(st["m"], m)
            if c == NC - 1:
                m_s[:, pl.ds(q0, NQ)] = jnp.broadcast_to(
                    jnp.max(st["m"], axis=0, keepdims=True), (8, NQ))

        def probs(t):
            u, c = divmod(t, NC)
            cols = pl.ds(col0 + u * NQ, NQ)
            if c == 0:
                st["mp"] = mp = m_s[:, cols]
            else:
                mp = jnp.minimum(st["mp"], st["l"] + jnp.inf)
            p = jnp.exp2(s_s[pl.ds(c * KC, KC), cols].reshape(KC // 8, 8, NQ) - mp[None])
            l = jnp.sum(p, axis=0)
            st["l"] = l if c == 0 else st["l"] + l
            st["p", t] = p.reshape(KC, NQ).astype(BF16)

        def values(t):
            u, c = divmod(t, NC)
            o = _dot(_unpack(vt_s[:, pl.ds(c * KC, KC)]), st.pop(("p", t)))
            st["o"] = o if c == 0 else st["o"] + o
            if c == NC - 1:
                inv = 1.0 / jnp.sum(st["l"], axis=0, keepdims=True)
                ot_s[_half(h_pv * DH, DH), pl.ds(col0 + u * NQ, NQ)] = _pack(st["o"] * inv)

        for t in range(nu * NC):
            if h_pv is not None:
                probs(t)
                values(t)
            if h_qk is not None:
                scores(t)

    def transpose_o(i):
        base = pl.multiple_of(i * TB, TB)
        o_s[_half(base, TB), :] = _pack(_unpack(ot_s[:, pl.ds(base, TB)]).T)

    def shifted(ref, t, off):
        n = HALO + RT
        full = ref[t, pl.ds(off, n), :]
        sub = lax.broadcasted_iota(jnp.int32, (n // 8 - 1, 8, 128), 1)
        out = [None] * WIN
        for s in range(SH):
            if s == 0:
                blk = full[8:]
            else:
                rot = pltpu.roll(full.reshape(n // 8, 8, 128), s * DIL, 1)
                blk = jnp.where(sub >= s * DIL, rot[1:], rot[:-1]).reshape(n - 8, 128)
            out[s] = blk[8:]
            out[s + SH] = blk[:RT]
        return out

    def window_weights(q, off, pos0):
        logits = None
        for t in range(NT):
            prod = [q[t] * k for k in shifted(kh_s, t, off)]
            logits = prod if t == 0 else [x + y for x, y in zip(logits, prod)]
        for w in range(WIN):
            acc = logits[w]
            acc = acc + pltpu.roll(acc, 2 * H, 1)
            acc = acc + pltpu.roll(acc, H, 1)
            if off < w * DIL:
                pos = pos0 + off + lax.broadcasted_iota(jnp.int32, (RT, 128), 0)
                acc = jnp.where(pos >= w * DIL, acc, MASKED)
            logits[w] = acc
        m = logits[0]
        for w in range(1, WIN):
            m = jnp.maximum(m, logits[w])
        p = [jnp.exp2(lg - m) for lg in logits]
        l = p[0]
        for w in range(1, WIN):
            l = l + p[w]
        inv = 1.0 / l
        return [pw * inv for pw in p]

    def window_values(p, off):
        out = []
        for t in range(NT):
            prod = [pw * v for pw, v in zip(p, shifted(vh_s, t, off))]
            acc = prod[0]
            for w in range(1, WIN):
                acc = acc + prod[w]
            out.append(acc.astype(BF16))
        return jnp.concatenate(out, axis=1)

    def window_attention(q, off, pos0):
        p = [window_weights([x[r:r + RT] for x in q], off + r, pos0) for r in range(0, TS, RT)]
        return jnp.concatenate(
            [window_values(p[r // RT], off + r) for r in range(0, TS, RT)], axis=0)

    def block(last, i, carry):
        base = pl.multiple_of(i * TB, TB)
        subs = range(TB // TS)
        start = [pl.multiple_of(base + a * TS, TS) for a in subs]

        if last:
            slot = i % 2

            @pl.when(i >= 2)
            def _():
                out_copy(i - 2, slot).wait()

        tail = pl.ds(TB, HALO)
        kh_s[:, pl.ds(0, HALO), :] = jnp.where(i > 0, kh_s[:, tail, :], 0.0)
        v_tail = vh_s[:, tail, :]

        x1 = [xres[pl.ds(start[a], TS), :]
              + _dot(_unpack(o_s[_half(start[a], TS), :]), _weights(awo)) for a in subs]
        transpose_o(jnp.minimum(i + 1, NB - 1))

        qs = []
        for a in subs:
            qkv = _dot(_layernorm(x1[a]), _weights(bwqkv))
            dst = pl.ds(HALO + a * TS, TS)
            qs.append([qkv[:, t * 128:(t + 1) * 128] * QSCALE for t in range(NT)])
            for t in range(NT):
                kh_s[t, dst, :] = qkv[:, (NT + t) * 128:(NT + t + 1) * 128]
                v = qkv[:, (2 * NT + t) * 128:(2 * NT + t + 1) * 128]
                vh_s[t, dst, :] = v
                if a == 0:
                    vh_s[t, pl.ds(0, HALO), :] = jnp.where(
                        i > 0, v_tail[t], jnp.broadcast_to(v[:1], (HALO, 128)))

        x2 = []
        for a in subs:
            x2.append(x1[a] + _dot(window_attention(qs[a], a * TS, base), _weights(bwo)))
            if last:
                out_s[slot, pl.ds(a * TS, TS), :] = x2[a].astype(BF16)
            else:
                xres[pl.ds(start[a], TS), :] = x2[a]

        if last:
            out_copy(i, slot).start()
        else:
            xn = [_layernorm(v) for v in x2]
            for a in subs:
                if a == len(subs) - 1:
                    project_kv(jnp.concatenate(xn, axis=0), base, TB)
                project_q(xn[a], start[a], TS)
        return carry

    def layer(li, carry):
        def scores_only(u, c):
            attention(0, None, pl.multiple_of(u * NQ, NQ), 1)
            return c

        def head(h, c):
            attention(h, h - 1, 0, NU)
            return c

        def values_only(u, c):
            attention(None, H - 1, pl.multiple_of(u * NQ, NQ), 1)
            return c

        lax.fori_loop(0, NU, scores_only, 0)
        lax.fori_loop(1, H, head, 0)
        lax.fori_loop(0, NU, values_only, 0)
        transpose_o(0)

        @pl.when(li == 0)
        def _():
            lax.fori_loop(0, NB, lambda i, c: block(False, i, c), 0)

        @pl.when(li == 1)
        def _():
            lax.fori_loop(0, NB, lambda i, c: block(True, i, c), 0)

        return carry

    lax.fori_loop(0, 2, layer, 0)
    out_copy(NB - 2, 0).wait()
    out_copy(NB - 1, 1).wait()


@jax.jit
def pallas_interleave_layers__grouped_kv_mqa__sliding_local_dilated__prompt_kernel(
    A_x: jax.Array,
    A_wq: jax.Array,
    A_wk: jax.Array,
    A_wv: jax.Array,
    A_wo: jax.Array,
    B_x: jax.Array,
    B_wqkv: jax.Array,
    B_wo: jax.Array,
):
    del B_x
    any_spec = pl.BlockSpec(memory_space=pl.ANY)
    out = pl.pallas_call(
        _kernel,
        in_specs=[any_spec] * 7,
        out_specs=any_spec,
        out_shape=jax.ShapeDtypeStruct((S, D), BF16),
        scratch_shapes=[
            pltpu.VMEM((S // 2, D), U32),
            pltpu.VMEM((S, D), F32),
            pltpu.VMEM((TF // 2, D), U32),
            pltpu.VMEM((NT, D // 2, 128), U32),
            pltpu.VMEM((DH, D), U32),
            pltpu.VMEM((NT, D // 2, 128), U32),
            pltpu.VMEM((3 * NT, D // 2, 128), U32),
            pltpu.VMEM((3 * NT, D // 2, 128), U32),
            pltpu.VMEM((NT, D // 2, 128), U32),
            pltpu.VMEM((NT, D // 2, 128), U32),
            pltpu.VMEM((D, 128), U32),
            pltpu.VMEM((NT, S // 2, 128), U32),
            pltpu.VMEM((4, S // 2, 128), U32),
            pltpu.VMEM((DH // 2, S), U32),
            pltpu.VMEM((S, S), F32),
            pltpu.VMEM((8, S), F32),
            pltpu.VMEM((D // 2, S), U32),
            pltpu.VMEM((S // 2, D), U32),
            pltpu.VMEM((NT, HALO + TB, 128), F32),
            pltpu.VMEM((NT, HALO + TB, 128), F32),
            pltpu.VMEM((2, TB, D), BF16),
            pltpu.SemaphoreType.DMA((5,)),
            pltpu.SemaphoreType.DMA((XC,)),
            pltpu.SemaphoreType.DMA((2,)),
        ],
        compiler_params=pltpu.CompilerParams(vmem_limit_bytes=120 * 1024 * 1024),
    )(A_x.reshape(S, D), A_wq, A_wk.T, A_wv.T, A_wo, B_wqkv, B_wo)
    return out.reshape(A_x.shape)
```

```python
import functools

import jax
import jax.numpy as jnp
from jax import lax
import jax.experimental.pallas as pl
import jax.experimental.pallas.tpu as pltpu

S = 2048
D = 1024
H = 32
DH = D // H
WIN = 8
DIL = 2
EPS = 1e-5
LOG2E = 1.4426950408889634
QSCALE = DH ** -0.5 * LOG2E
MASKED = -1e9 * LOG2E

NQ = 512
NU = S // NQ
KC = 128
NC = S // KC
TF = 128
TB = 256
TS = 64
RT = 16
NB = S // TB
XB = (0, TF, 6 * TF, S)
NP = 12
HALO = 16
NT = D // 128
SH = 8 // DIL

F32 = jnp.float32
BF16 = jnp.bfloat16
U32 = jnp.uint32


def _dot(a, b):
    return jnp.dot(a, b, preferred_element_type=F32)


def _dot_nt(a, b):
    return lax.dot_general(a, b, (((1,), (1,)), ((), ())), preferred_element_type=F32)


def _pack(x):
    return pltpu.bitcast(x.astype(BF16), U32)


def _unpack(x):
    return pltpu.bitcast(x, BF16)


def _weights(ref, t0=0, t1=NT):
    return _unpack(jnp.concatenate([ref[t] for t in range(t0, t1)], axis=1))


def _layernorm(x):
    m = jnp.mean(x, axis=-1, keepdims=True)
    c = x - m
    v = jnp.mean(c * c, axis=-1, keepdims=True)
    return (c * lax.rsqrt(v + EPS)).astype(BF16)


def _aligned(start, size):
    return pl.ds(start if isinstance(start, int) else pl.multiple_of(start, size), size)


def _half(start, size):
    return _aligned(start // 2, size // 2)


def _kernel(x_hbm, awq_hbm, awkt_hbm, awvt_hbm, awo_hbm, bwqkv_hbm, bwo_hbm, out_hbm,
            xin, xres, xn_s, awq, awkvt, awo, bwqkv_raw, bwqkv, bwo_raw, bwo, tr_s,
            q_s, k4_s, vt_s, s_s, m_s, ot_s, o_s, kh_s, vh_s, out_s,
            sem_in, sem_x, sem_out):
    def x_copy(i):
        rows = pl.ds(XB[i], XB[i + 1] - XB[i])
        return pltpu.make_async_copy(x_hbm.at[rows], xin.bitcast(BF16).at[rows], sem_x.at[i])

    def tile_copies(src, dst, sem, t0=0, t1=NT):
        return [pltpu.make_async_copy(src.at[:, pl.ds(t * 128, 128)], dst.bitcast(BF16).at[t], sem)
                for t in range(t0, t1)]

    def out_copy(i, slot):
        return pltpu.make_async_copy(
            out_s.at[slot], out_hbm.at[_aligned(i * TB, TB)], sem_out.at[slot])

    def project_q(xn, base, n, t0=0, t1=NT):
        q = _pack(_dot(xn, _weights(awq, t0, t1)) * QSCALE)
        for t in range(t0, t1):
            q_s[t, _half(base, n), :] = q[:, (t - t0) * 128:(t - t0 + 1) * 128]

    def project_kv(xn, base, n, layer):
        kvt = _dot_nt(_unpack(awkvt[...]), xn)
        vt_s[layer, :, pl.ds(base, n)] = _pack(kvt[DH:])
        krep = jnp.concatenate([kvt[:DH]] * 4, axis=0).T
        lane = lax.broadcasted_iota(jnp.int32, (n, 128), 1)
        for j in range(4):
            k4_s[j, _half(base, n), :] = _pack(jnp.where(lane // DH == j, krep, 0.0))

    def permute_qkv(n):
        sec = n // 4
        r = _aligned((n % 4) * 128, 128)
        for t in range(NT):
            tr_s[pl.ds(t * 128, 128), :] = bwqkv_raw[sec * NT + t, r, :].T
        for t in range(NT):
            blk = jnp.concatenate(
                [tr_s[pl.ds(4 * t + e, H, stride=DH), :] for e in range(4)], axis=0)
            bwqkv[sec * NT + t, r, :] = blk.T

    def permute_wo(t):
        for dp in range(DH // 2):
            ev = bwo_raw[t, pl.ds(dp, H // 2, stride=DH), :]
            od = bwo_raw[t, pl.ds(DH // 2 + dp, H // 2, stride=DH), :]
            bwo[t, pl.ds(dp * H, H // 2), :] = (ev & 0xFFFF) | (od << 16)
            bwo[t, pl.ds(dp * H + H // 2, H // 2), :] = (ev >> 16) | (od & U32(0xFFFF0000))

    nf = S // TF
    p0 = nf - NP
    mid = p0 + NP // 3
    head_cps = [
        pltpu.make_async_copy(src, awkvt.bitcast(BF16).at[pl.ds(e * DH, DH)], sem_in.at[0])
        for e, src in enumerate((awkt_hbm, awvt_hbm))] + tile_copies(awq_hbm, awq, sem_in.at[0])
    fetch = [
        ([x_copy(1)], -1, XB[1] // TF),
        (tile_copies(bwqkv_hbm, bwqkv_raw, sem_in.at[1]), -1, p0),
        ([x_copy(2)], 0, XB[2] // TF - 1),
        (tile_copies(bwqkv_hbm, bwqkv_raw, sem_in.at[2], NT, 3 * NT), 0, mid),
        (tile_copies(bwo_hbm, bwo_raw, sem_in.at[3])
         + tile_copies(awo_hbm, awo, sem_in.at[4]), mid, nf),
    ]

    def advance_fetch(n):
        for cps, start, _ in fetch:
            if start == n:
                for cp in cps:
                    cp.start()
        for cps, _, need in fetch:
            if need == n:
                for cp in cps:
                    cp.wait()

    def first_norm(i):
        base = pl.multiple_of(i * TF, TF)
        x = _unpack(xin[_half(base, TF), :]).astype(F32)
        xres[pl.ds(base, TF), :] = x
        xn_s[...] = pltpu.bitcast(_layernorm(x), U32)

    def first(lo, hi, permute):
        events = sorted({n for _, start, need in fetch for n in (start, need) if lo < n < hi})

        def body(i, carry):
            for n in events:
                pl.when(i == n)(functools.partial(advance_fetch, n))
            base = pl.multiple_of(i * TF, TF)
            xn = _unpack(xn_s[...])
            if permute:
                permute_qkv(i - p0)
            project_q(xn, base, TF, 0, NT // 2)
            project_kv(xn, base, TF, 0)
            project_q(xn, base, TF, NT // 2, NT)
            first_norm(jnp.minimum(i + 1, nf - 1))
            return carry

        advance_fetch(lo)
        lax.fori_loop(lo, hi, body, 0)

    x_copy(0).start()
    for cp in head_cps:
        cp.start()
    x_copy(0).wait()
    first_norm(0)
    for cp in head_cps:
        cp.wait()
    advance_fetch(-1)
    first(0, p0, False)
    first(p0, nf, True)
    advance_fetch(nf)

    def attention_steps(layer, h_qk, h_pv, col0, nu, nq):
        st = {}

        def after(mp, l):
            return jnp.minimum(mp, l + jnp.inf) if h_qk is not None else mp

        def probs(t):
            u, c = divmod(t, NC)
            cols = pl.ds(col0 + u * nq, nq)
            if c == 0:
                st["mp"] = m_s[:, cols]
            mp = st["mp"] if t == 0 else after(st["mp"], st["lp"] if c > 1 else st["l"])
            p = jnp.exp2(s_s[pl.ds(c * KC, KC), cols].reshape(KC // 8, 8, nq) - mp[None])
            st["lp"] = l = st.get("l")
            for r in range(0, KC // 8, 2):
                l = p[r] + p[r + 1] if c == r == 0 else l + (p[r] + p[r + 1])
            st["l"] = l
            st["p"] = p.reshape(KC, nq).astype(BF16)
            if c == NC - 1:
                st["inv"] = 1.0 / jnp.sum(l, axis=0, keepdims=True)

        def scores(t):
            u, c = divmod(t, NC)
            q0 = col0 + u * nq
            s = _dot_nt(_unpack(k4_s[h_qk % 4, _half(c * KC, KC), :]),
                        _unpack(q_s[h_qk // 4, _half(q0, nq), :]))
            s_s[pl.ds(c * KC, KC), pl.ds(q0, nq)] = s
            m = jnp.max(s.reshape(KC // 8, 8, nq), axis=0)
            st["m"] = m if c == 0 else jnp.maximum(st["m"], m)
            if c == NC - 1:
                m_s[:, pl.ds(q0, nq)] = jnp.broadcast_to(
                    jnp.max(st["m"], axis=0, keepdims=True), (8, nq))

        def values(t):
            u, c = divmod(t, NC)
            o = _dot(_unpack(vt_s[layer, :, pl.ds(c * KC, KC)]), st["p"])
            st["o"] = o if c == 0 else st["o"] + o
            if c == NC - 1:
                ot_s[_half(h_pv * DH, DH), pl.ds(col0 + u * nq, nq)] = _pack(st["o"] * st["inv"])

        for t in range(nu * NC):
            if h_pv is not None:
                probs(t)
            if h_qk is not None:
                scores(t)
            if h_pv is not None:
                values(t)
            yield

    def attention(*args):
        for _ in attention_steps(*args):
            pass

    def transpose_o(base, t0=0, t1=NT):
        o_s[_half(base, TB), pl.ds(t0 * 128, (t1 - t0) * 128)] = _pack(
            _unpack(ot_s[_half(t0 * 128, (t1 - t0) * 128), pl.ds(base, TB)]).T)

    def shifted(ref, t, off):
        n = HALO + RT
        full = ref[t, pl.ds(off, n), :]
        sub = lax.broadcasted_iota(jnp.int32, (n // 8 - 1, 8, 128), 1)
        out = [None] * WIN
        for s in range(SH):
            if s == 0:
                blk = full[8:]
            else:
                rot = pltpu.roll(full.reshape(n // 8, 8, 128), s * DIL, 1)
                blk = jnp.where(sub >= s * DIL, rot[1:], rot[:-1]).reshape(n - 8, 128)
            out[s] = blk[8:]
            out[s + SH] = blk[:RT]
        return out

    def window_weights(q, off, pos0):
        logits = None
        for t in range(NT):
            prod = [q[t] * k for k in shifted(kh_s, t, off)]
            logits = prod if t == 0 else [x + y for x, y in zip(logits, prod)]
        for w in range(WIN):
            acc = logits[w]
            acc = acc + pltpu.roll(acc, 2 * H, 1)
            acc = acc + pltpu.roll(acc, H, 1)
            if off < w * DIL:
                pos = pos0 + off + lax.broadcasted_iota(jnp.int32, (RT, 128), 0)
                acc = jnp.where(pos >= w * DIL, acc, MASKED)
            logits[w] = acc
        m = logits[0]
        for w in range(1, WIN):
            m = jnp.maximum(m, logits[w])
        p = [jnp.exp2(lg - m) for lg in logits]
        l = p[0]
        for w in range(1, WIN):
            l = l + p[w]
        inv = 1.0 / l
        return [pw * inv for pw in p]

    def window_values(p, off):
        out = []
        for t in range(NT):
            prod = [pw * v for pw, v in zip(p, shifted(vh_s, t, off))]
            acc = prod[0]
            for w in range(1, WIN):
                acc = acc + prod[w]
            out.append(acc.astype(BF16))
        return jnp.concatenate(out, axis=1)

    def window_attention(q, off, pos0):
        p = [window_weights([x[r:r + RT] for x in q], off + r, pos0) for r in range(0, TS, RT)]
        return jnp.concatenate(
            [window_values(p[r // RT], off + r) for r in range(0, TS, RT)], axis=0)

    def block(last, i, carry):
        base = pl.multiple_of(i * TB, TB)
        subs = range(TB // TS)
        start = [pl.multiple_of(base + a * TS, TS) for a in subs]

        if last:
            slot = i % 2

            @pl.when(i >= 2)
            def _():
                out_copy(i - 2, slot).wait()

        tail = pl.ds(TB, HALO)
        kh_s[:, pl.ds(0, HALO), :] = jnp.where(i > 0, kh_s[:, tail, :], 0.0)
        v_tail = vh_s[:, tail, :]

        ahead = pl.multiple_of(jnp.minimum(i + 1, NB - 1) * TB, TB)
        steps = attention_steps(int(last), None, H - 1, ahead, 1, TB)

        def advance():
            next(steps, None)
            next(steps, None)

        x1 = []
        for a in subs:
            x1.append(xres[pl.ds(start[a], TS), :]
                      + _dot(_unpack(o_s[_half(start[a], TS), :]), _weights(awo)))
            advance()

        qs = []
        for a in subs:
            xn = _layernorm(x1[a])
            qkv = []
            for e in range(3):
                qkv.append(_dot(xn, _weights(bwqkv, e * NT, (e + 1) * NT)))
                advance()
            q, k, v = ([y[:, t * 128:(t + 1) * 128] for t in range(NT)] for y in qkv)
            dst = pl.ds(HALO + a * TS, TS)
            qs.append([y * QSCALE for y in q])
            for t in range(NT):
                kh_s[t, dst, :] = k[t]
                vh_s[t, dst, :] = v[t]
                if a == 0:
                    vh_s[t, pl.ds(0, HALO), :] = jnp.where(
                        i > 0, v_tail[t], jnp.broadcast_to(v[t][:1], (HALO, 128)))
        for _ in steps:
            pass
        transpose_o(ahead)

        x2 = []
        for a in subs:
            x2.append(x1[a] + _dot(window_attention(qs[a], a * TS, base), _weights(bwo)))
            if last:
                out_s[slot, pl.ds(a * TS, TS), :] = x2[a].astype(BF16)
            else:
                xres[pl.ds(start[a], TS), :] = x2[a]

        if last:
            out_copy(i, slot).start()
        else:
            xn = [_layernorm(v) for v in x2]
            for a in subs:
                if a == len(subs) - 1:
                    project_kv(jnp.concatenate(xn, axis=0), base, TB, 1)
                project_q(xn[a], start[a], TS)
        return carry

    def layer(li, carry):
        def scores_only(u, c):
            for e in range(NT // NU):
                permute_wo(u * (NT // NU) + e)
            attention(li, 0, None, pl.multiple_of(u * NQ, NQ), 1, NQ)
            return c

        def head(h, c):
            attention(li, h, h - 1, 0, NU, NQ)
            return c

        lax.fori_loop(0, NU, scores_only, 0)
        lax.fori_loop(1, H, head, 0)
        transpose_o(0, 0, NT - 1)
        attention(li, None, H - 1, 0, 1, TB)
        transpose_o(0, NT - 1, NT)

        @pl.when(li == 0)
        def _():
            lax.fori_loop(0, NB, lambda i, c: block(False, i, c), 0)

        @pl.when(li == 1)
        def _():
            lax.fori_loop(0, NB, lambda i, c: block(True, i, c), 0)

        return carry

    lax.fori_loop(0, 2, layer, 0)
    out_copy(NB - 2, 0).wait()
    out_copy(NB - 1, 1).wait()


@jax.jit
def pallas_interleave_layers__grouped_kv_mqa__sliding_local_dilated__prompt_kernel(
    A_x: jax.Array,
    A_wq: jax.Array,
    A_wk: jax.Array,
    A_wv: jax.Array,
    A_wo: jax.Array,
    B_x: jax.Array,
    B_wqkv: jax.Array,
    B_wo: jax.Array,
):
    del B_x
    any_spec = pl.BlockSpec(memory_space=pl.ANY)
    out = pl.pallas_call(
        _kernel,
        in_specs=[any_spec] * 7,
        out_specs=any_spec,
        out_shape=jax.ShapeDtypeStruct((S, D), BF16),
        scratch_shapes=[
            pltpu.VMEM((S // 2, D), U32),
            pltpu.VMEM((S, D), F32),
            pltpu.VMEM((TF // 2, D), U32),
            pltpu.VMEM((NT, D // 2, 128), U32),
            pltpu.VMEM((DH, D), U32),
            pltpu.VMEM((NT, D // 2, 128), U32),
            pltpu.VMEM((3 * NT, D // 2, 128), U32),
            pltpu.VMEM((3 * NT, D // 2, 128), U32),
            pltpu.VMEM((NT, D // 2, 128), U32),
            pltpu.VMEM((NT, D // 2, 128), U32),
            pltpu.VMEM((D, 128), U32),
            pltpu.VMEM((NT, S // 2, 128), U32),
            pltpu.VMEM((4, S // 2, 128), U32),
            pltpu.VMEM((2, DH // 2, S), U32),
            pltpu.VMEM((S, S), F32),
            pltpu.VMEM((8, S), F32),
            pltpu.VMEM((D // 2, S), U32),
            pltpu.VMEM((S // 2, D), U32),
            pltpu.VMEM((NT, HALO + TB, 128), F32),
            pltpu.VMEM((NT, HALO + TB, 128), F32),
            pltpu.VMEM((2, TB, D), BF16),
            pltpu.SemaphoreType.DMA((5,)),
            pltpu.SemaphoreType.DMA((3,)),
            pltpu.SemaphoreType.DMA((2,)),
        ],
        compiler_params=pltpu.CompilerParams(vmem_limit_bytes=120 * 1024 * 1024),
    )(A_x.reshape(S, D), A_wq, A_wk.T, A_wv.T, A_wo, B_wqkv, B_wo)
    return out.reshape(A_x.shape)
```

```python
import functools

import jax
import jax.numpy as jnp
from jax import lax
import jax.experimental.pallas as pl
import jax.experimental.pallas.tpu as pltpu

S = 2048
D = 1024
H = 32
DH = D // H
WIN = 8
DIL = 2
EPS = 1e-5
LOG2E = 1.4426950408889634
QSCALE = DH ** -0.5 * LOG2E
MASKED = -1e9 * LOG2E

NQ = 512
NU = S // NQ
KC = 128
NC = S // KC
TF = 128
TB = 256
TS = 64
RT = 16
NB = S // TB
XB = (0, TF, 6 * TF, S)
NP = 12
HALO = 16
NT = D // 128
SH = 8 // DIL

F32 = jnp.float32
BF16 = jnp.bfloat16
U32 = jnp.uint32


def _dot(a, b):
    return jnp.dot(a, b, preferred_element_type=F32)


def _dot_nt(a, b):
    return lax.dot_general(a, b, (((1,), (1,)), ((), ())), preferred_element_type=F32)


def _pack(x):
    return pltpu.bitcast(x.astype(BF16), U32)


def _unpack(x):
    return pltpu.bitcast(x, BF16)


def _weights(ref, t0=0, t1=NT):
    return _unpack(jnp.concatenate([ref[t] for t in range(t0, t1)], axis=1))


def _layernorm(x):
    m = jnp.mean(x, axis=-1, keepdims=True)
    c = x - m
    v = jnp.mean(c * c, axis=-1, keepdims=True)
    return (c * lax.rsqrt(v + EPS)).astype(BF16)


def _aligned(start, size):
    return pl.ds(start if isinstance(start, int) else pl.multiple_of(start, size), size)


def _half(start, size):
    return _aligned(start // 2, size // 2)


def _kernel(x_hbm, awq_hbm, awkt_hbm, awvt_hbm, awo_hbm, bwqkv_hbm, bwo_hbm, out_hbm,
            xin, xres, xn_s, awq, awkvt, awo, bwqkv_raw, bwqkv, bwo_raw, bwo, qt_s,
            q_s, k4_s, vt_s, s_s, m_s, ot_s, o_s, kh_s, vh_s, out_s,
            sem_in, sem_x, sem_out):
    def x_copy(i):
        rows = pl.ds(XB[i], XB[i + 1] - XB[i])
        return pltpu.make_async_copy(x_hbm.at[rows], xin.bitcast(BF16).at[rows], sem_x.at[i])

    def tile_copies(src, dst, sem, t0=0, t1=NT):
        return [pltpu.make_async_copy(src.at[:, pl.ds(t * 128, 128)], dst.bitcast(BF16).at[t], sem)
                for t in range(t0, t1)]

    def out_copy(i, slot):
        return pltpu.make_async_copy(
            out_s.at[slot], out_hbm.at[_aligned(i * TB, TB)], sem_out.at[slot])

    def project_q(xn, base, n, t0=0, t1=NT):
        q = _pack(_dot(xn, _weights(awq, t0, t1)) * QSCALE)
        for t in range(t0, t1):
            q_s[t, _half(base, n), :] = q[:, (t - t0) * 128:(t - t0 + 1) * 128]

    def project_kv(xn, base, n, layer):
        kvt = _dot_nt(_unpack(awkvt[...]), xn)
        vt_s[layer, :, pl.ds(base, n)] = _pack(kvt[DH:])
        krep = jnp.concatenate([kvt[:DH]] * 4, axis=0).T
        lane = lax.broadcasted_iota(jnp.int32, (n, 128), 1)
        for j in range(4):
            k4_s[j, _half(base, n), :] = _pack(jnp.where(lane // DH == j, krep, 0.0))

    def permute_qkv(n):
        t0 = n // 4 * NT
        r = _aligned((n % 4) * 128, 128)
        cols = jnp.concatenate([bwqkv_raw[t0 + t, r, :].T for t in range(NT)], axis=0)
        cols = jnp.swapaxes(cols.reshape(H, DH, 128), 0, 1).reshape(D, 128)
        for t in range(NT):
            bwqkv[t0 + t, r, :] = cols[t * 128:(t + 1) * 128].T

    def permute_wo(t):
        x = bwo_raw[t].reshape(H // 2, 2, DH // 2, 128)
        ev, od = x[:, 0], x[:, 1]
        lo = jnp.swapaxes((ev & 0xFFFF) | (od << 16), 0, 1)
        hi = jnp.swapaxes((ev >> 16) | (od & U32(0xFFFF0000)), 0, 1)
        bwo[t] = jnp.stack([lo, hi], axis=1).reshape(D // 2, 128)

    nf = S // TF
    p0 = nf - NP
    mid = p0 + NP // 3
    head_cps = [
        pltpu.make_async_copy(src, awkvt.bitcast(BF16).at[pl.ds(e * DH, DH)], sem_in.at[0])
        for e, src in enumerate((awkt_hbm, awvt_hbm))] + tile_copies(awq_hbm, awq, sem_in.at[0])
    fetch = [
        ([x_copy(1)], -1, XB[1] // TF),
        (tile_copies(bwqkv_hbm, bwqkv_raw, sem_in.at[1]), -1, p0),
        ([x_copy(2)], 0, XB[2] // TF - 1),
        (tile_copies(bwqkv_hbm, bwqkv_raw, sem_in.at[2], NT, 3 * NT), 0, mid),
        (tile_copies(bwo_hbm, bwo_raw, sem_in.at[3])
         + tile_copies(awo_hbm, awo, sem_in.at[4]), mid, nf),
    ]

    def advance_fetch(n):
        for cps, start, _ in fetch:
            if start == n:
                for cp in cps:
                    cp.start()
        for cps, _, need in fetch:
            if need == n:
                for cp in cps:
                    cp.wait()

    def first_norm(i):
        base = pl.multiple_of(i * TF, TF)
        x = _unpack(xin[_half(base, TF), :]).astype(F32)
        xres[pl.ds(base, TF), :] = x
        xn_s[...] = pltpu.bitcast(_layernorm(x), U32)

    def first(lo, hi, permute):
        events = sorted({n for _, start, need in fetch for n in (start, need) if lo < n < hi})

        def body(i, carry):
            for n in events:
                pl.when(i == n)(functools.partial(advance_fetch, n))
            base = pl.multiple_of(i * TF, TF)
            xn = _unpack(xn_s[...])
            if permute:
                permute_qkv(i - p0)
            project_q(xn, base, TF, 0, NT // 2)
            project_kv(xn, base, TF, 0)
            project_q(xn, base, TF, NT // 2, NT)
            first_norm(jnp.minimum(i + 1, nf - 1))
            return carry

        advance_fetch(lo)
        lax.fori_loop(lo, hi, body, 0)

    x_copy(0).start()
    for cp in head_cps:
        cp.start()
    x_copy(0).wait()
    first_norm(0)
    for cp in head_cps:
        cp.wait()
    advance_fetch(-1)
    first(0, p0, False)
    first(p0, nf, True)
    advance_fetch(nf)

    def attention_steps(layer, h_qk, h_pv, col0, nu, nq):
        st = {}

        def after(mp, l):
            return jnp.minimum(mp, l + jnp.inf) if h_qk is not None else mp

        def probs(t):
            u, c = divmod(t, NC)
            cols = pl.ds(col0 + u * nq, nq)
            if c == 0:
                st["mp"] = m_s[:, cols]
            mp = st["mp"] if t == 0 else after(st["mp"], st["lp"] if c > 1 else st["l"])
            p = jnp.exp2(s_s[pl.ds(c * KC, KC), cols].reshape(KC // 8, 8, nq) - mp[None])
            st["lp"] = l = st.get("l")
            for r in range(0, KC // 8, 4):
                part = (p[r] + p[r + 1]) + (p[r + 2] + p[r + 3])
                l = part if c == r == 0 else l + part
            st["l"] = l
            st["p"] = p.reshape(KC, nq).astype(BF16)
            if c == NC - 1:
                st["inv"] = 1.0 / jnp.sum(l, axis=0, keepdims=True)

        def scores(t):
            u, c = divmod(t, NC)
            q0 = col0 + u * nq
            k = _unpack(k4_s[h_qk % 4, _half(c * KC, KC), :])
            if h_pv is not None and u == 0:
                s = _dot(k, _unpack(qt_s[...]))
            else:
                s = _dot_nt(k, _unpack(q_s[h_qk // 4, _half(q0, nq), :]))
            s_s[pl.ds(c * KC, KC), pl.ds(q0, nq)] = s
            m = jnp.max(s.reshape(KC // 8, 8, nq), axis=0)
            st["m"] = m if c == 0 else jnp.maximum(st["m"], m)
            if c == NC - 1:
                m_s[:, pl.ds(q0, nq)] = jnp.broadcast_to(
                    jnp.max(st["m"], axis=0, keepdims=True), (8, nq))

        def values(t):
            u, c = divmod(t, NC)
            o = _dot(_unpack(vt_s[layer, :, pl.ds(c * KC, KC)]), st["p"])
            st["o"] = o if c == 0 else st["o"] + o
            if c == NC - 1:
                ot_s[_half(h_pv * DH, DH), pl.ds(col0 + u * nq, nq)] = _pack(st["o"] * st["inv"])

        for t in range(nu * NC):
            if h_pv is not None:
                probs(t)
            if h_qk is not None:
                scores(t)
            if h_pv is not None:
                values(t)
            yield

    def attention(*args):
        for _ in attention_steps(*args):
            pass

    def transpose_q(h):
        qt_s[...] = _pack(_unpack(q_s[jnp.minimum(h, H - 1) // 4, _half(0, NQ), :]).T)

    def transpose_o(base, t0=0, t1=NT):
        o_s[_half(base, TB), pl.ds(t0 * 128, (t1 - t0) * 128)] = _pack(
            _unpack(ot_s[_half(t0 * 128, (t1 - t0) * 128), pl.ds(base, TB)]).T)

    def shifted(ref, t, off):
        n = HALO + RT
        full = ref[t, pl.ds(off, n), :]
        sub = lax.broadcasted_iota(jnp.int32, (n // 8 - 1, 8, 128), 1)
        out = [None] * WIN
        for s in range(SH):
            if s == 0:
                blk = full[8:]
            else:
                rot = pltpu.roll(full.reshape(n // 8, 8, 128), s * DIL, 1)
                blk = jnp.where(sub >= s * DIL, rot[1:], rot[:-1]).reshape(n - 8, 128)
            out[s] = blk[8:]
            out[s + SH] = blk[:RT]
        return out

    def window_weights(q, off, pos0):
        logits = None
        for t in range(NT):
            prod = [q[t] * k for k in shifted(kh_s, t, off)]
            logits = prod if t == 0 else [x + y for x, y in zip(logits, prod)]
        for w in range(WIN):
            acc = logits[w]
            acc = acc + pltpu.roll(acc, 2 * H, 1)
            acc = acc + pltpu.roll(acc, H, 1)
            if off < w * DIL:
                pos = pos0 + off + lax.broadcasted_iota(jnp.int32, (RT, 128), 0)
                acc = jnp.where(pos >= w * DIL, acc, MASKED)
            logits[w] = acc
        m = logits[0]
        for w in range(1, WIN):
            m = jnp.maximum(m, logits[w])
        p = [jnp.exp2(lg - m) for lg in logits]
        l = p[0]
        for w in range(1, WIN):
            l = l + p[w]
        inv = 1.0 / l
        return [pw * inv for pw in p]

    def window_values(p, off):
        out = []
        for t in range(NT):
            prod = [pw * v for pw, v in zip(p, shifted(vh_s, t, off))]
            acc = prod[0]
            for w in range(1, WIN):
                acc = acc + prod[w]
            out.append(acc.astype(BF16))
        return jnp.concatenate(out, axis=1)

    def window_attention(q, off, pos0):
        p = [window_weights([x[r:r + RT] for x in q], off + r, pos0) for r in range(0, TS, RT)]
        return jnp.concatenate(
            [window_values(p[r // RT], off + r) for r in range(0, TS, RT)], axis=0)

    def block(last, i, carry):
        base = pl.multiple_of(i * TB, TB)
        subs = range(TB // TS)
        start = [pl.multiple_of(base + a * TS, TS) for a in subs]

        if last:
            slot = i % 2

            @pl.when(i >= 2)
            def _():
                out_copy(i - 2, slot).wait()

        tail = pl.ds(TB, HALO)
        kh_s[:, pl.ds(0, HALO), :] = jnp.where(i > 0, kh_s[:, tail, :], 0.0)
        v_tail = vh_s[:, tail, :]

        ahead = pl.multiple_of(jnp.minimum(i + 1, NB - 1) * TB, TB)
        steps = attention_steps(int(last), None, H - 1, ahead, 1, TB)

        def advance():
            next(steps, None)
            next(steps, None)

        x1 = []
        for a in subs:
            x1.append(xres[pl.ds(start[a], TS), :]
                      + _dot(_unpack(o_s[_half(start[a], TS), :]), _weights(awo)))
            advance()

        qs = []
        for a in subs:
            xn = _layernorm(x1[a])
            qkv = []
            for e in range(3):
                qkv.append(_dot(xn, _weights(bwqkv, e * NT, (e + 1) * NT)))
                advance()
            q, k, v = ([y[:, t * 128:(t + 1) * 128] for t in range(NT)] for y in qkv)
            dst = pl.ds(HALO + a * TS, TS)
            qs.append([y * QSCALE for y in q])
            for t in range(NT):
                kh_s[t, dst, :] = k[t]
                vh_s[t, dst, :] = v[t]
                if a == 0:
                    vh_s[t, pl.ds(0, HALO), :] = jnp.where(
                        i > 0, v_tail[t], jnp.broadcast_to(v[t][:1], (HALO, 128)))
        for _ in steps:
            pass
        transpose_o(ahead)

        x2 = []
        for a in subs:
            x2.append(x1[a] + _dot(window_attention(qs[a], a * TS, base), _weights(bwo)))
            if last:
                out_s[slot, pl.ds(a * TS, TS), :] = x2[a].astype(BF16)
            else:
                xres[pl.ds(start[a], TS), :] = x2[a]

        if last:
            out_copy(i, slot).start()
        else:
            xn = [_layernorm(v) for v in x2]
            for a in subs:
                if a == len(subs) - 1:
                    project_kv(jnp.concatenate(xn, axis=0), base, TB, 1)
                project_q(xn[a], start[a], TS)
        return carry

    def layer(li, carry):
        def scores_only(u, c):
            for e in range(NT // NU):
                permute_wo(u * (NT // NU) + e)
            attention(li, 0, None, pl.multiple_of(u * NQ, NQ), 1, NQ)
            transpose_q(1)
            return c

        def head(h, c):
            attention(li, h, h - 1, 0, NU, NQ)
            transpose_q(h + 1)
            return c

        lax.fori_loop(0, NU, scores_only, 0)
        lax.fori_loop(1, H, head, 0)
        transpose_o(0, 0, NT - 1)
        attention(li, None, H - 1, 0, 1, TB)
        transpose_o(0, NT - 1, NT)

        @pl.when(li == 0)
        def _():
            lax.fori_loop(0, NB, lambda i, c: block(False, i, c), 0)

        @pl.when(li == 1)
        def _():
            lax.fori_loop(0, NB, lambda i, c: block(True, i, c), 0)

        return carry

    lax.fori_loop(0, 2, layer, 0)
    out_copy(NB - 2, 0).wait()
    out_copy(NB - 1, 1).wait()


@jax.jit
def pallas_interleave_layers__grouped_kv_mqa__sliding_local_dilated__prompt_kernel(
    A_x: jax.Array,
    A_wq: jax.Array,
    A_wk: jax.Array,
    A_wv: jax.Array,
    A_wo: jax.Array,
    B_x: jax.Array,
    B_wqkv: jax.Array,
    B_wo: jax.Array,
):
    del B_x
    any_spec = pl.BlockSpec(memory_space=pl.ANY)
    out = pl.pallas_call(
        _kernel,
        in_specs=[any_spec] * 7,
        out_specs=any_spec,
        out_shape=jax.ShapeDtypeStruct((S, D), BF16),
        scratch_shapes=[
            pltpu.VMEM((S // 2, D), U32),
            pltpu.VMEM((S, D), F32),
            pltpu.VMEM((TF // 2, D), U32),
            pltpu.VMEM((NT, D // 2, 128), U32),
            pltpu.VMEM((DH, D), U32),
            pltpu.VMEM((NT, D // 2, 128), U32),
            pltpu.VMEM((3 * NT, D // 2, 128), U32),
            pltpu.VMEM((3 * NT, D // 2, 128), U32),
            pltpu.VMEM((NT, D // 2, 128), U32),
            pltpu.VMEM((NT, D // 2, 128), U32),
            pltpu.VMEM((64, NQ), U32),
            pltpu.VMEM((NT, S // 2, 128), U32),
            pltpu.VMEM((4, S // 2, 128), U32),
            pltpu.VMEM((2, DH // 2, S), U32),
            pltpu.VMEM((S, S), F32),
            pltpu.VMEM((8, S), F32),
            pltpu.VMEM((D // 2, S), U32),
            pltpu.VMEM((S // 2, D), U32),
            pltpu.VMEM((NT, HALO + TB, 128), F32),
            pltpu.VMEM((NT, HALO + TB, 128), F32),
            pltpu.VMEM((2, TB, D), BF16),
            pltpu.SemaphoreType.DMA((5,)),
            pltpu.SemaphoreType.DMA((3,)),
            pltpu.SemaphoreType.DMA((2,)),
        ],
        compiler_params=pltpu.CompilerParams(vmem_limit_bytes=120 * 1024 * 1024),
    )(A_x.reshape(S, D), A_wq, A_wk.T, A_wv.T, A_wo, B_wqkv, B_wo)
    return out.reshape(A_x.shape)
```

```python
import functools

import jax
import jax.numpy as jnp
from jax import lax
import jax.experimental.pallas as pl
import jax.experimental.pallas.tpu as pltpu

S = 2048
D = 1024
H = 32
DH = D // H
WIN = 8
DIL = 2
EPS = 1e-5
LOG2E = 1.4426950408889634
QSCALE = DH ** -0.5 * LOG2E
MASKED = -1e9 * LOG2E

NQ = 512
NU = S // NQ
KC = 128
NC = S // KC
TF = 128
TB = 256
TS = 64
RT = 16
NB = S // TB
XB = (0, 2 * TF, 6 * TF, S)
NP = 12
HALO = 16
NT = D // 128
SH = 8 // DIL

F32 = jnp.float32
BF16 = jnp.bfloat16
U32 = jnp.uint32


def _dot(a, b):
    return jnp.dot(a, b, preferred_element_type=F32)


def _dot_nt(a, b):
    return lax.dot_general(a, b, (((1,), (1,)), ((), ())), preferred_element_type=F32)


def _pack(x):
    return pltpu.bitcast(x.astype(BF16), U32)


def _unpack(x):
    return pltpu.bitcast(x, BF16)


def _weights(ref, t0=0, t1=NT):
    if ref.dtype == BF16:
        return ref[:, pl.ds(t0 * 128, (t1 - t0) * 128)]
    return _unpack(jnp.concatenate([ref[t] for t in range(t0, t1)], axis=1))


def _layernorm(x):
    m = jnp.mean(x, axis=-1, keepdims=True)
    c = x - m
    v = jnp.mean(c * c, axis=-1, keepdims=True)
    return (c * lax.rsqrt(v + EPS)).astype(BF16)


def _aligned(start, size):
    return pl.ds(start if isinstance(start, int) else pl.multiple_of(start, size), size)


def _half(start, size):
    return _aligned(start // 2, size // 2)


def _kernel(x_hbm, awq_hbm, awkt_hbm, awvt_hbm, awo_hbm, bwqkv_hbm, bwo_hbm, out_hbm,
            xin, xres, xn_s, awq, awkvt, awo_raw, awo, bwqkv_raw, bwqkv, bwo_raw, bwo, qt_s,
            q_s, k4_s, vt_s, s_s, m_s, ot_s, o_s, kh_s, vh_s, out_s,
            sem_in, sem_x, sem_out):
    def x_copy(i):
        rows = pl.ds(XB[i], XB[i + 1] - XB[i])
        return pltpu.make_async_copy(x_hbm.at[rows], xin.at[rows], sem_x.at[i])

    def tile_copies(src, dst, sem):
        return [pltpu.make_async_copy(src.at[:, pl.ds(t * 128, 128)], dst.at[t], sem)
                for t in range(NT)]

    def qkv_copy(lo, hi, sem):
        cols = pl.ds(lo * D, (hi - lo) * D)
        return pltpu.make_async_copy(bwqkv_hbm.at[:, cols], bwqkv_raw.at[:, cols], sem)

    def out_copy(i, slot, a):
        return pltpu.make_async_copy(
            out_s.at[slot, pl.ds(a * TS, TS)], out_hbm.at[_aligned(i * TB + a * TS, TS)],
            sem_out.at[slot])

    def project_q(xn, base, n, t0=0, t1=NT):
        q = _pack(_dot(xn, _weights(awq, t0, t1)) * QSCALE)
        for t in range(t0, t1):
            q_s[t, _half(base, n), :] = q[:, (t - t0) * 128:(t - t0 + 1) * 128]

    def project_kv(xn, base, n, layer):
        kvt = _dot_nt(awkvt[...], xn)
        vt_s[layer, :, pl.ds(base, n)] = _pack(kvt[DH:])
        krep = jnp.concatenate([kvt[:DH]] * 4, axis=0).T
        lane = lax.broadcasted_iota(jnp.int32, (n, 128), 1)
        for j in range(4):
            k4_s[j, _half(base, n), :] = _pack(jnp.where(lane // DH == j, krep, 0.0))

    def permute_qkv(n):
        t0 = n // 4 * NT
        r = _aligned((n % 4) * 128, 128)
        cols = jnp.concatenate([pltpu.bitcast(
            bwqkv_raw[_aligned((n % 4) * 256, 256), _aligned((t0 + t) * 128, 128)], U32).T for t in range(NT)], axis=0)
        cols = jnp.swapaxes(cols.reshape(H, DH, 128), 0, 1).reshape(D, 128)
        for t in range(NT):
            bwqkv[t0 + t, r, :] = cols[t * 128:(t + 1) * 128].T

    def prepare_weights(t):
        awo[t] = pltpu.bitcast(awo_raw[t], U32)
        x = pltpu.bitcast(bwo_raw[t], U32).reshape(H // 2, 2, DH // 2, 128)
        ev, od = x[:, 0], x[:, 1]
        lo = jnp.swapaxes((ev & 0xFFFF) | (od << 16), 0, 1)
        hi = jnp.swapaxes((ev >> 16) | (od & U32(0xFFFF0000)), 0, 1)
        bwo[t] = jnp.stack([lo, hi], axis=1).reshape(D // 2, 128)

    nf = S // TF
    p0 = nf - NP
    mid = p0 + NP // 3
    head_cps = [
        pltpu.make_async_copy(src, awkvt.at[pl.ds(e * DH, DH)], sem_in.at[0])
        for e, src in enumerate((awkt_hbm, awvt_hbm))] + [
        pltpu.make_async_copy(awq_hbm, awq, sem_in.at[0])]
    fetch = [
        ([x_copy(1)], -1, XB[1] // TF - 1),
        ([qkv_copy(0, 1, sem_in.at[1])], -1, p0),
        ([x_copy(2)], 0, XB[2] // TF - 1),
        ([qkv_copy(1, 3, sem_in.at[2])], 0, mid),
        (tile_copies(bwo_hbm, bwo_raw, sem_in.at[3]), mid, nf),
        (tile_copies(awo_hbm, awo_raw, sem_in.at[4]), mid, nf),
    ]

    def advance_fetch(n):
        for cps, start, _ in fetch:
            if start == n:
                for cp in cps:
                    cp.start()
        for cps, _, need in fetch:
            if need == n:
                for cp in cps:
                    cp.wait()

    def first_norm(i):
        base = pl.multiple_of(i * TF, TF)
        x = xin[pl.ds(base, TF), :].astype(F32)
        xres[pl.ds(base, TF), :] = x
        xn_s[...] = pltpu.bitcast(_layernorm(x), U32)

    def first(lo, hi, permute):
        events = sorted({n for _, start, need in fetch for n in (start, need) if lo < n < hi})

        def body(i, carry):
            for n in events:
                pl.when(i == n)(functools.partial(advance_fetch, n))
            base = pl.multiple_of(i * TF, TF)
            xn = _unpack(xn_s[...])
            if permute:
                permute_qkv(i - p0)
            project_q(xn, base, TF, 0, NT // 2)
            project_kv(xn, base, TF, 0)
            project_q(xn, base, TF, NT // 2, NT)
            first_norm(jnp.minimum(i + 1, nf - 1))
            return carry

        advance_fetch(lo)
        lax.fori_loop(lo, hi, body, 0)

    x_copy(0).start()
    for cp in head_cps:
        cp.start()
    x_copy(0).wait()
    first_norm(0)
    for cp in head_cps:
        cp.wait()
    advance_fetch(-1)
    first(0, p0, False)
    first(p0, nf, True)
    advance_fetch(nf)

    def attention_steps(layer, h_qk, h_pv, col0, nu, nq):
        st = {}

        def after(mp, l):
            return jnp.where(l < 0, l, mp) if h_qk is not None else mp

        def probs(t):
            u, c = divmod(t, NC)
            cols = pl.ds(col0 + u * nq, nq)
            if c == 0:
                st["mp"] = m_s[:, cols]
            mp = st["mp"] if t == 0 else after(st["mp"], st["lp"] if c > 1 else st["l"])
            p = jnp.exp2(s_s[pl.ds(c * KC, KC), cols].reshape(KC // 8, 8, nq) - mp[None])
            st["lp"] = l = st.get("l")
            for r in range(0, KC // 8, 4):
                part = (p[r] + p[r + 1]) + (p[r + 2] + p[r + 3])
                l = part if c == r == 0 else l + part
            st["l"] = l
            st["p"] = p.reshape(KC, nq).astype(BF16)
            if c == NC - 1:
                st["inv"] = 1.0 / jnp.sum(l, axis=0, keepdims=True)

        def scores(t):
            u, c = divmod(t, NC)
            q0 = col0 + u * nq
            k = _unpack(k4_s[h_qk % 4, _half(c * KC, KC), :])
            if h_pv is not None and u == 0:
                s = _dot(k, _unpack(qt_s[...]))
            else:
                s = _dot_nt(k, _unpack(q_s[h_qk // 4, _half(q0, nq), :]))
            s_s[pl.ds(c * KC, KC), pl.ds(q0, nq)] = s
            m = jnp.max(s.reshape(KC // 8, 8, nq), axis=0)
            st["m"] = m if c == 0 else jnp.maximum(st["m"], m)
            if c == NC - 1:
                m_s[:, pl.ds(q0, nq)] = jnp.broadcast_to(
                    jnp.max(st["m"], axis=0, keepdims=True), (8, nq))

        def values(t):
            u, c = divmod(t, NC)
            o = _dot(_unpack(vt_s[layer, :, pl.ds(c * KC, KC)]), st["p"])
            st["o"] = o if c == 0 else st["o"] + o
            if c == NC - 1:
                ot_s[_half(h_pv * DH, DH), pl.ds(col0 + u * nq, nq)] = _pack(st["o"] * st["inv"])

        for t in range(nu * NC):
            if h_pv is not None:
                probs(t)
            if h_qk is not None:
                scores(t)
            if h_pv is not None:
                values(t)
            yield

    def attention(*args):
        for _ in attention_steps(*args):
            pass

    def transpose_q(h):
        qt_s[...] = _pack(_unpack(q_s[jnp.minimum(h, H - 1) // 4, _half(0, NQ), :]).T)

    def transpose_o(base, t0=0, t1=NT):
        o_s[_half(base, TB), pl.ds(t0 * 128, (t1 - t0) * 128)] = _pack(
            _unpack(ot_s[_half(t0 * 128, (t1 - t0) * 128), pl.ds(base, TB)]).T)

    def shifted(ref, t, off):
        n = HALO + RT
        full = ref[t, pl.ds(off, n), :]
        sub = lax.broadcasted_iota(jnp.int32, (n // 8 - 1, 8, 128), 1)
        out = [None] * WIN
        for s in range(SH):
            if s == 0:
                blk = full[8:]
            else:
                rot = pltpu.roll(full.reshape(n // 8, 8, 128), s * DIL, 1)
                blk = jnp.where(sub >= s * DIL, rot[1:], rot[:-1]).reshape(n - 8, 128)
            out[s] = blk[8:]
            out[s + SH] = blk[:RT]
        return out

    def window_weights(q, off, pos0):
        logits = None
        for t in range(NT):
            prod = [q[t] * k for k in shifted(kh_s, t, off)]
            logits = prod if t == 0 else [x + y for x, y in zip(logits, prod)]
        for w in range(WIN):
            acc = logits[w]
            acc = acc + pltpu.roll(acc, 2 * H, 1)
            acc = acc + pltpu.roll(acc, H, 1)
            if off < w * DIL:
                pos = pos0 + off + lax.broadcasted_iota(jnp.int32, (RT, 128), 0)
                acc = jnp.where(pos >= w * DIL, acc, MASKED)
            logits[w] = acc
        m = logits[0]
        for w in range(1, WIN):
            m = jnp.maximum(m, logits[w])
        p = [jnp.exp2(lg - m) for lg in logits]
        l = p[0]
        for w in range(1, WIN):
            l = l + p[w]
        inv = 1.0 / l
        return [pw * inv for pw in p]

    def window_values(p, off):
        out = []
        for t in range(NT):
            prod = [pw * v for pw, v in zip(p, shifted(vh_s, t, off))]
            acc = prod[0]
            for w in range(1, WIN):
                acc = acc + prod[w]
            out.append(acc.astype(BF16))
        return jnp.concatenate(out, axis=1)

    def window_attention(q, off, pos0):
        p = [window_weights([x[r:r + RT] for x in q], off + r, pos0) for r in range(0, TS, RT)]
        return jnp.concatenate(
            [window_values(p[r // RT], off + r) for r in range(0, TS, RT)], axis=0)

    def block(last, i, carry):
        base = pl.multiple_of(i * TB, TB)
        subs = range(TB // TS)
        start = [pl.multiple_of(base + a * TS, TS) for a in subs]

        if last:
            slot = i % 2

            @pl.when(i >= 2)
            def _():
                for a in subs:
                    out_copy(i - 2, slot, a).wait()

        tail = pl.ds(TB, HALO)
        kh_s[:, pl.ds(0, HALO), :] = jnp.where(i > 0, kh_s[:, tail, :], 0.0)
        v_tail = vh_s[:, tail, :]

        ahead = pl.multiple_of(jnp.minimum(i + 1, NB - 1) * TB, TB)
        steps = attention_steps(int(last), None, H - 1, ahead, 1, TB)

        def advance():
            next(steps, None)
            next(steps, None)

        x1 = []
        for a in subs:
            x1.append(xres[pl.ds(start[a], TS), :]
                      + _dot(_unpack(o_s[_half(start[a], TS), :]), _weights(awo)))
            advance()

        qs = []
        for a in subs:
            xn = _layernorm(x1[a])
            qkv = []
            for e in range(3):
                qkv.append(_dot(xn, _weights(bwqkv, e * NT, (e + 1) * NT)))
                advance()
            q, k, v = ([y[:, t * 128:(t + 1) * 128] for t in range(NT)] for y in qkv)
            dst = pl.ds(HALO + a * TS, TS)
            qs.append([y * QSCALE for y in q])
            for t in range(NT):
                kh_s[t, dst, :] = k[t]
                vh_s[t, dst, :] = v[t]
                if a == 0:
                    vh_s[t, pl.ds(0, HALO), :] = jnp.where(
                        i > 0, v_tail[t], jnp.broadcast_to(v[t][:1], (HALO, 128)))
        for _ in steps:
            pass
        transpose_o(ahead)

        x2 = []
        for a in subs:
            x2.append(x1[a] + _dot(window_attention(qs[a], a * TS, base), _weights(bwo)))
            if last:
                out_s[slot, pl.ds(a * TS, TS), :] = x2[a].astype(BF16)
                out_copy(i, slot, a).start()
            else:
                xres[pl.ds(start[a], TS), :] = x2[a]

        if not last:
            xn = [_layernorm(v) for v in x2]
            for a in subs:
                if a == len(subs) - 1:
                    project_kv(jnp.concatenate(xn, axis=0), base, TB, 1)
                project_q(xn[a], start[a], TS)
        return carry

    kh_s[:, pl.ds(TB, HALO), :] = jnp.zeros((NT, HALO, 128), F32)
    vh_s[:, pl.ds(TB, HALO), :] = jnp.zeros((NT, HALO, 128), F32)

    def layer(li, carry):
        def scores_only(prepare, u, c):
            for e in range(NT // NU if prepare else 0):
                prepare_weights(u * (NT // NU) + e)
            attention(li, 0, None, pl.multiple_of(u * NQ, NQ), 1, NQ)
            transpose_q(1)
            return c

        def head(h, c):
            attention(li, h, h - 1, 0, NU, NQ)
            transpose_q(h + 1)
            return c

        for first_layer in (True, False):
            @pl.when((li == 0) == first_layer)
            def _():
                lax.fori_loop(0, NU, functools.partial(scores_only, first_layer), 0)

        lax.fori_loop(1, H, head, 0)
        transpose_o(0, 0, NT - 1)
        attention(li, None, H - 1, 0, 1, TB)
        transpose_o(0, NT - 1, NT)

        @pl.when(li == 0)
        def _():
            lax.fori_loop(0, NB, lambda i, c: block(False, i, c), 0)

        @pl.when(li == 1)
        def _():
            lax.fori_loop(0, NB, lambda i, c: block(True, i, c), 0)

        return carry

    lax.fori_loop(0, 2, layer, 0)
    for i in (NB - 2, NB - 1):
        for a in range(TB // TS):
            out_copy(i, i % 2, a).wait()


@jax.jit
def pallas_interleave_layers__grouped_kv_mqa__sliding_local_dilated__prompt_kernel(
    A_x: jax.Array,
    A_wq: jax.Array,
    A_wk: jax.Array,
    A_wv: jax.Array,
    A_wo: jax.Array,
    B_x: jax.Array,
    B_wqkv: jax.Array,
    B_wo: jax.Array,
):
    del B_x
    any_spec = pl.BlockSpec(memory_space=pl.ANY)
    out = pl.pallas_call(
        _kernel,
        in_specs=[any_spec] * 7,
        out_specs=any_spec,
        out_shape=jax.ShapeDtypeStruct((S, D), BF16),
        scratch_shapes=[
            pltpu.VMEM((S, D), BF16),
            pltpu.VMEM((S, D), F32),
            pltpu.VMEM((TF // 2, D), U32),
            pltpu.VMEM((D, D), BF16),
            pltpu.VMEM((2 * DH, D), BF16),
            pltpu.VMEM((NT, D, 128), BF16),
            pltpu.VMEM((NT, D // 2, 128), U32),
            pltpu.VMEM((D, 3 * D), BF16),
            pltpu.VMEM((3 * NT, D // 2, 128), U32),
            pltpu.VMEM((NT, D, 128), BF16),
            pltpu.VMEM((NT, D // 2, 128), U32),
            pltpu.VMEM((64, NQ), U32),
            pltpu.VMEM((NT, S // 2, 128), U32),
            pltpu.VMEM((4, S // 2, 128), U32),
            pltpu.VMEM((2, DH // 2, S), U32),
            pltpu.VMEM((S, S), F32),
            pltpu.VMEM((8, S), F32),
            pltpu.VMEM((D // 2, S), U32),
            pltpu.VMEM((S // 2, D), U32),
            pltpu.VMEM((NT, HALO + TB, 128), F32),
            pltpu.VMEM((NT, HALO + TB, 128), F32),
            pltpu.VMEM((2, TB, D), BF16),
            pltpu.SemaphoreType.DMA((5,)),
            pltpu.SemaphoreType.DMA((3,)),
            pltpu.SemaphoreType.DMA((2,)),
        ],
        compiler_params=pltpu.CompilerParams(vmem_limit_bytes=120 * 1024 * 1024),
    )(A_x.reshape(S, D), A_wq, A_wk.T, A_wv.T, A_wo, B_wqkv, B_wo)
    return out.reshape(A_x.shape)
```
